```python
import jax
import jax.numpy as jnp

def _softmax(x, axis=-1):
    return jax.nn.softmax(x, axis=axis)

def _gelu(x):
    return jax.nn.gelu(x, approximate=True)

def _silu(x):
    return jax.nn.silu(x)

def _sigmoid(x):
    return jax.nn.sigmoid(x)

def _layernorm(x, axis=-1, eps=1e-05):
    m = jnp.mean(x, axis=axis, keepdims=True)
    v = jnp.var(x, axis=axis, keepdims=True)
    return (x - m) / jnp.sqrt(v + eps)

def _scatter_add(tgt, idx, src, axis=0):
    return tgt.at[idx].add(src)

def _segment_sum(src, seg, n):
    return jax.ops.segment_sum(src, seg, n)

class _Rng:

    def __init__(self, key):
        self._k = key

    def _next(self):
        self._k, sub = jax.random.split(self._k)
        return sub

    def normal(self, shape):
        return jax.random.normal(self._next(), shape, dtype=jnp.bfloat16)

    def randint(self, lo, hi, shape):
        return jax.random.randint(self._next(), shape, lo, hi, dtype=jnp.int32)

    def uniform(self, shape, lo=0.0, hi=1.0):
        return jax.random.uniform(self._next(), shape, jnp.bfloat16, lo, hi)

    def permutation(self, n):
        return jax.random.permutation(self._next(), n)
kernel_name = 'adaLN_cond__memory_aug_recurrent_mem_tr__dense_activation_gelu__prompt'

def setup_inputs():
    _rng = _Rng(jax.random.key(int.from_bytes(__import__("os").urandom(4), "little")))
    _w = lambda a: (lambda t: t.astype(jnp.bfloat16) if jnp.issubdtype(t.dtype, jnp.floating) else t)(jnp.asarray(a))

    def _A_setup():
        B, S, Dm = (1, 2048, 1024)
        H, Dh = (32, 128)
        M, seg = (8, 32)
        seg = min(seg, S)
        S = S // seg * seg
        return {'x': _w((lambda *s: _rng.normal(s) * 0.05)(B, S, Dm)), 'mem0': _w((lambda *s: _rng.normal(s) * 0.05)(B, M, Dm)), 'Wq': _w((lambda *s: _rng.normal(s) * 0.05)(Dm, H, Dh) * Dm ** (-0.5)), 'Wk': _w((lambda *s: _rng.normal(s) * 0.05)(Dm, H, Dh) * Dm ** (-0.5)), 'Wv': _w((lambda *s: _rng.normal(s) * 0.05)(Dm, H, Dh) * Dm ** (-0.5)), 'Wo': _w((lambda *s: _rng.normal(s) * 0.05)(H, Dh, Dm) * (H * Dh) ** (-0.5)), 'seg_len': seg}
    _A_in = _A_setup()

    def _B_setup():
        B, S, D, F = (1, 2048, 1024, 3584)
        return {'x': _w((lambda *s: _rng.normal(s) * 0.05)(B, S, D)), 'w1': _w((lambda *s: _rng.normal(s) * 0.05)(D, F) * D ** (-0.5)), 'b1': _w((lambda *s: _rng.normal(s) * 0.05)(F) * 0.01), 'w2': _w((lambda *s: _rng.normal(s) * 0.05)(F, D) * F ** (-0.5)), 'b2': _w((lambda *s: _rng.normal(s) * 0.05)(D) * 0.01)}
    _B_in = _B_setup()
    return {'A_x': _A_in['x'], 'A_mem0': _A_in['mem0'], 'A_Wq': _A_in['Wq'], 'A_Wk': _A_in['Wk'], 'A_Wv': _A_in['Wv'], 'A_Wo': _A_in['Wo'], 'A_seg_len': _A_in['seg_len'], 'B_x': _B_in['x'], 'B_w1': _B_in['w1'], 'B_b1': _B_in['b1'], 'B_w2': _B_in['w2'], 'B_b2': _B_in['b2'], 'c': _w((lambda *s: _rng.normal(s) * 0.05)(1, 1024)), 'w_mod': _w((lambda *s: _rng.normal(s) * 0.05)(1024, 6 * 1024) * 1024 ** (-0.5))}

def reference(A_x, A_mem0, A_Wq, A_Wk, A_Wv, A_Wo, A_seg_len, B_x, B_w1, B_b1, B_w2, B_b2, c, w_mod):

    def _A_ref(x, mem0, Wq, Wk, Wv, Wo, seg_len):
        B, S, Dm = x.shape
        H, Dh = (Wq.shape[1], Wq.shape[2])
        M = mem0.shape[1]
        scale = Dh ** (-0.5)
        n_seg = S // seg_len
        L = M + seg_len
        idx = jnp.arange(L)
        mask = (idx[:, None] < M) | (idx[:, None] >= idx[None, :])
        mem = mem0
        outs = []
        for s in range(n_seg):
            xs = x[:, s * seg_len:(s + 1) * seg_len, :].copy()
            h = jnp.concatenate([mem, xs], axis=1)
            q = jnp.einsum('btd,dhe->bhte', h, Wq)
            k = jnp.einsum('btd,dhe->bhte', h, Wk)
            v = jnp.einsum('btd,dhe->bhte', h, Wv)
            scores = jnp.einsum('bhqe,bhke->bhqk', q, k) * scale
            scores = jnp.where(mask[None, None], scores, -1000000000.0)
            p = _softmax(scores, axis=-1)
            o = jnp.einsum('bhqk,bhke->bhqe', p, v)
            o = jnp.einsum('bhte,hed->btd', o, Wo)
            mem = o[:, :M, :].copy()
            outs.append(o[:, M:, :])
        return jnp.concatenate(outs, axis=1)

    def _B_ref(x, w1, b1, w2, b2):
        h = jnp.einsum('bsd,df->bsf', x, w1) + b1
        h = _gelu(h)
        return jnp.einsum('bsf,fd->bsd', h, w2) + b2
    x = A_x
    mod = (_silu(c) @ w_mod).reshape(c.shape[0], 6, 1, -1)
    sa, ca, ga, sb, cb, gb = (mod[:, 0].copy(), mod[:, 1].copy(), mod[:, 2].copy(), mod[:, 3].copy(), mod[:, 4].copy(), mod[:, 5].copy())
    h = _layernorm(x, axis=-1) * (1 + ca) + sa
    x = x + ga * _A_ref(h, A_mem0, A_Wq, A_Wk, A_Wv, A_Wo, A_seg_len)
    h = _layernorm(x, axis=-1) * (1 + cb) + sb
    x = x + gb * _B_ref(h, B_w1, B_b1, B_w2, B_b2)
    return x
```

```python
import functools

import jax
import jax.numpy as jnp
from jax import lax
import jax.experimental.pallas as pl
import jax.experimental.pallas.tpu as pltpu

F32 = jnp.float32
BF16 = jnp.bfloat16
U32 = jnp.uint32

_PROF = False


def _scope(name):
    import contextlib
    return jax.named_scope(name) if _PROF else contextlib.nullcontext()


_EPS = 1e-5
_NEG = -1e30


def _ln(x):
    m = jnp.mean(x, axis=-1, keepdims=True)
    xc = x - m
    v = jnp.mean(xc * xc, axis=-1, keepdims=True)
    return xc * lax.rsqrt(v + _EPS)


def _dot(a, b):
    return jnp.dot(a, b, preferred_element_type=F32)


def _dot_nt(a, b):
    return lax.dot_general(a, b, (((1,), (1,)), ((), ())), preferred_element_type=F32)


def _make_kernel(S, D, H, E, M, SEG, F):
    NSEG = S // SEG
    HE = H * E
    RIDE = 24
    XTRA = SEG - RIDE
    NX = NSEG * XTRA
    L = M + SEG
    LP = 48
    scale = float(E) ** -0.5
    MODC = 2 * D

    def kernel(x_hbm, mem0_ref, wq_hbm, wk_hbm, wv_hbm, wo_hbm, w1_hbm, b1_ref,
               w2_hbm, b2_ref, c_ref, wmod_hbm, out_hbm,
               wq_s, wk_s, wv_s, wo_s, stage, w1_s, w2_s, wm_s, x_s, h_s, mod_s,
               qe_s, ke_s, ve_s, oxp_s, oe_s, ob_s, ka_s, va_s, qm_s, qx_s, sems, osems):
        def cp(src, dst, i):
            return pltpu.make_async_copy(src, dst, sems.at[i])

        cp_wm0 = cp(wmod_hbm.at[:, pl.ds(0, MODC)], wm_s, 0)
        cp_x = cp(x_hbm, x_s, 1)
        cp_q = cp(wq_hbm, stage.at[0], 2)
        cp_k = cp(wk_hbm, stage.at[1], 3)
        cp_v = cp(wv_hbm, stage.at[0], 4)
        cp_o = [cp(wo_hbm.at[:, pl.ds(j * 128, 128)], wo_s.at[j], 5 + j) for j in range(D // 128)]
        nd = 5 + D // 128
        cp_wm1 = cp(wmod_hbm.at[:, pl.ds(MODC, MODC)], wm_s, nd)
        cp_wm2 = cp(wmod_hbm.at[:, pl.ds(2 * MODC, MODC)], wm_s, nd + 1)
        cp_w1 = cp(w1_hbm, w1_s, nd + 2)
        cp_w2 = cp(w2_hbm, w2_s, nd + 3)

        cp_wm0.start()
        cp_x.start()
        cp_q.start()
        cp_k.start()

        c = c_ref[...].astype(F32).astype(BF16).astype(F32)
        sc = (c * jax.nn.sigmoid(c)).astype(BF16)
        sc = jnp.broadcast_to(sc, (8, D))

        def mod_chunk(j):
            r = _dot(sc, wm_s[...])
            mod_s[:, pl.ds(j * MODC, MODC)] = r.astype(BF16).astype(F32)

        with _scope("wait_wm0"):
            cp_wm0.wait()
        mod_chunk(0)
        cp_wm1.start()

        with _scope("wait_x"):
            cp_x.wait()
        sa = mod_s[0:1, 0:D]
        ca = mod_s[0:1, D:2 * D]

        def ln1_body(i, _):
            r = pl.multiple_of(i * 128, 128)
            xv = x_s[pl.ds(r, 128), :].astype(F32)
            h_s[pl.ds(r, 128), :] = _ln(xv) * (1.0 + ca) + sa
            return 0

        with _scope("ln1"):
            lax.fori_loop(0, S // 128, ln1_body, 0)

        def retile(slot, dst):
            src = stage.at[slot].bitcast(U32)

            def body(t, _):
                base = pl.multiple_of(t * (8 * H), 8 * H)
                blk = src.at[pl.ds(base, 8 * H), :]
                r = pl.multiple_of(t * 8, 8)
                for hp in range(H // 2):
                    a = blk[pl.ds(hp, 8, stride=H), :]
                    b = blk[pl.ds(H // 2 + hp, 8, stride=H), :]
                    dst[2 * hp, pl.ds(r, 8), :] = (a & U32(0xFFFF)) | (b << 16)
                    dst[2 * hp + 1, pl.ds(r, 8), :] = (a >> 16) | (b & U32(0xFFFF0000))
                return 0

            lax.fori_loop(0, D // 16, body, 0)

        def wtile(ref, h):
            return pltpu.bitcast(ref[h], BF16)

        def extra_proj(w_ref, dst):
            for blk in range(NX // 128):
                segs = 128 // XTRA
                he = jnp.concatenate(
                    [h_s[pl.ds((blk * segs + s) * SEG + RIDE, XTRA), :] for s in range(segs)],
                    axis=0).astype(BF16)

                def body(h, _):
                    dst[h, pl.ds(blk * 128, 128), :] = _dot(he, wtile(w_ref, h)).astype(BF16)
                    return 0

                lax.fori_loop(0, H, body, 0)

        with _scope("wait_q"):
            cp_q.wait()
        with _scope("retile_q"):
            retile(0, wq_s)
        cp_v.start()
        with _scope("extra_q"):
            extra_proj(wq_s, qe_s)
        with _scope("wait_k"):
            cp_k.wait()
        with _scope("retile_k"):
            retile(1, wk_s)
        for d in cp_o:
            d.start()
        with _scope("extra_k"):
            extra_proj(wk_s, ke_s)
        with _scope("wait_v"):
            cp_v.wait()
        with _scope("retile_v"):
            retile(0, wv_s)
        cp_w1.start()
        cp_w2.start()
        with _scope("extra_v"):
            extra_proj(wv_s, ve_s)
        for d in cp_o:
            d.wait()
        cp_wm1.wait()
        mod_chunk(1)
        cp_wm2.start()

        ga = mod_s[0:1, 2 * D:3 * D]

        oxp_s[...] = jnp.zeros(oxp_s.shape, F32)
        colm = lax.broadcasted_iota(jnp.int32, (M, LP), 1)
        mask_m = colm < L
        rowx = lax.broadcasted_iota(jnp.int32, (SEG, LP), 0)
        colx = lax.broadcasted_iota(jnp.int32, (SEG, LP), 1)
        mask_x = colx <= rowx + M
        zpad = jnp.zeros((LP - L, E), F32)

        def softmax(s, mask):
            s = jnp.where(mask, s, _NEG)
            mx = jnp.max(s, axis=-1, keepdims=True)
            p = jnp.exp(s - mx)
            return p / jnp.sum(p, axis=-1, keepdims=True)

        def step(s, mem):
            r0 = pl.multiple_of(s * SEG, SEG)
            lhs = jnp.concatenate([mem, h_s[pl.ds(r0, RIDE), :]], axis=0).astype(BF16)
            e0 = pl.multiple_of(s * XTRA, XTRA)
            for h in range(H):
                q = _dot(lhs, wtile(wq_s, h))
                k = _dot(lhs, wtile(wk_s, h))
                v = _dot(lhs, wtile(wv_s, h))
                ke = ke_s[h, pl.ds(e0, XTRA), :].astype(F32)
                ve = ve_s[h, pl.ds(e0, XTRA), :].astype(F32)
                qe = qe_s[h, pl.ds(e0, XTRA), :].astype(F32)
                ka_s[h] = jnp.concatenate([k, ke, zpad], axis=0).astype(BF16)
                va_s[h] = jnp.concatenate([v, ve, zpad], axis=0).astype(BF16)
                qm_s[h] = q[0:M]
                qx_s[h] = jnp.concatenate([q[M:], qe], axis=0).astype(BF16)
            sms = [_dot_nt(qm_s[h].astype(BF16), ka_s[h]) * scale for h in range(H)]
            pms = [softmax(sm, mask_m).astype(BF16) for sm in sms]
            oms = [_dot(pms[h], va_s[h]) for h in range(H)]
            sxs = [_dot_nt(qx_s[h], ka_s[h]) * scale for h in range(H)]
            pxs = [softmax(sx, mask_x).astype(BF16) for sx in sxs]
            oxs = [_dot(pxs[h], va_s[h]) for h in range(H)]
            om = jnp.concatenate(oms, axis=1)
            lhs2 = jnp.concatenate([om, oxp_s[...]], axis=0).astype(BF16)
            outs = [_dot(lhs2, wo_s[j]) for j in range(D // 128)]
            out = jnp.concatenate(outs, axis=1)
            rp = pl.multiple_of(jnp.maximum(s - 1, 0) * SEG, SEG)
            xv = x_s[pl.ds(rp, RIDE), :].astype(F32)
            h_s[pl.ds(rp, RIDE), :] = xv + ga * out[M:]
            ox = jnp.concatenate(oxs, axis=1)
            oxp_s[...] = ox[0:RIDE]
            oe_s[pl.ds(e0, XTRA), :] = ox[RIDE:].astype(BF16)
            return out[0:M].astype(BF16).astype(F32)

        with _scope("loop"):
            lax.fori_loop(0, NSEG, step, mem0_ref[...].astype(F32))

        cp_w1.wait()
        cp_w2.wait()
        cp_wm2.wait()
        mod_chunk(2)

        lhs2 = jnp.concatenate([jnp.zeros((M, HE), F32), oxp_s[...]], axis=0).astype(BF16)
        out = jnp.concatenate([_dot(lhs2, wo_s[j]) for j in range(D // 128)], axis=1)
        rp = (NSEG - 1) * SEG
        h_s[pl.ds(rp, RIDE), :] = x_s[pl.ds(rp, RIDE), :].astype(F32) + ga * out[M:]

        for blk in range(NX // 128):
            segs = 128 // XTRA
            oe = oe_s[pl.ds(blk * 128, 128), :]
            out = jnp.concatenate([_dot(oe, wo_s[j]) for j in range(D // 128)], axis=1)
            for s in range(segs):
                r = (blk * segs + s) * SEG + RIDE
                h_s[pl.ds(r, XTRA), :] = (x_s[pl.ds(r, XTRA), :].astype(F32)
                                          + ga * out[s * XTRA:(s + 1) * XTRA])

        sb = mod_s[0:1, 3 * D:4 * D]
        cb = mod_s[0:1, 4 * D:5 * D]
        gb = mod_s[0:1, 5 * D:6 * D]
        b2 = b2_ref[...].astype(F32)
        BM = 256
        FC = 512
        NB = S // BM

        def out_copy(i, slot):
            return pltpu.make_async_copy(
                ob_s.at[slot], out_hbm.at[pl.ds(pl.multiple_of(i * BM, BM), BM), :], osems.at[slot])

        def ffn_body(i, _):
            slot = i % 2
            r = pl.multiple_of(i * BM, BM)
            x1 = h_s[pl.ds(r, BM), :]
            hb = (_ln(x1) * (1.0 + cb) + sb).astype(BF16)
            acc = jnp.zeros((BM, D), F32)
            for f in range(F // FC):
                h1 = _dot(hb, w1_s[:, f * FC:(f + 1) * FC]) + b1_ref[:, f * FC:(f + 1) * FC].astype(F32)
                g = jax.nn.gelu(h1, approximate=True).astype(BF16)
                acc = acc + _dot(g, w2_s[f * FC:(f + 1) * FC, :])
            res = x1 + gb * (acc + b2)

            @pl.when(i >= 2)
            def _():
                out_copy(i - 2, slot).wait()

            ob_s[slot] = res.astype(BF16)
            out_copy(i, slot).start()
            return 0

        with _scope("ffn"):
            lax.fori_loop(0, NB, ffn_body, 0)
        out_copy(NB - 2, (NB - 2) % 2).wait()
        out_copy(NB - 1, (NB - 1) % 2).wait()

    return kernel


@functools.partial(jax.jit, static_argnames=("A_seg_len",))
def _impl(A_x, A_mem0, A_Wq, A_Wk, A_Wv, A_Wo, B_w1, B_b1, B_w2, B_b2, c, w_mod, A_seg_len):
    B, S, D = A_x.shape
    H, E = A_Wq.shape[1], A_Wq.shape[2]
    M = A_mem0.shape[1]
    F = B_w1.shape[1]
    SEG = A_seg_len
    assert B == 1 and E == 128 and M == 8 and SEG == 32
    NX = (S // SEG) * 8
    kernel = _make_kernel(S, D, H, E, M, SEG, F)
    any_spec = pl.BlockSpec(memory_space=pl.ANY)
    vmem_spec = pl.BlockSpec(memory_space=pltpu.VMEM)
    out = pl.pallas_call(
        kernel,
        out_shape=jax.ShapeDtypeStruct((S, D), A_x.dtype),
        in_specs=[any_spec, vmem_spec, any_spec, any_spec, any_spec, any_spec, any_spec,
                  vmem_spec, any_spec, vmem_spec, vmem_spec, any_spec],
        out_specs=any_spec,
        scratch_shapes=[
            pltpu.VMEM((H, D // 2, E), U32),
            pltpu.VMEM((H, D // 2, E), U32),
            pltpu.VMEM((H, D // 2, E), U32),
            pltpu.VMEM((D // 128, H * E, 128), BF16),
            pltpu.VMEM((2, D * H, E), BF16),
            pltpu.VMEM((D, F), BF16),
            pltpu.VMEM((F, D), BF16),
            pltpu.VMEM((D, 2 * D), BF16),
            pltpu.VMEM((S, D), BF16),
            pltpu.VMEM((S, D), F32),
            pltpu.VMEM((8, 6 * D), F32),
            pltpu.VMEM((H, NX, E), BF16),
            pltpu.VMEM((H, NX, E), BF16),
            pltpu.VMEM((H, NX, E), BF16),
            pltpu.VMEM((24, H * E), F32),
            pltpu.VMEM((NX, H * E), BF16),
            pltpu.VMEM((2, 256, D), BF16),
            pltpu.VMEM((H, 48, E), BF16),
            pltpu.VMEM((H, 48, E), BF16),
            pltpu.VMEM((H, 8, E), F32),
            pltpu.VMEM((H, 32, E), BF16),
            pltpu.SemaphoreType.DMA((20,)),
            pltpu.SemaphoreType.DMA((2,)),
        ],
        compiler_params=pltpu.CompilerParams(vmem_limit_bytes=120 * 1024 * 1024),
    )(A_x.reshape(S, D), A_mem0.reshape(M, D),
      A_Wq.reshape(D * H, E), A_Wk.reshape(D * H, E), A_Wv.reshape(D * H, E),
      A_Wo.reshape(H * E, D), B_w1, B_b1.reshape(1, F), B_w2, B_b2.reshape(1, D), c, w_mod)
    return out.reshape(B, S, D)


def pallas_adaLN_cond__memory_aug_recurrent_mem_tr__dense_activation_gelu__prompt_kernel(
        A_x, A_mem0, A_Wq, A_Wk, A_Wv, A_Wo, A_seg_len, B_x, B_w1, B_b1, B_w2, B_b2, c, w_mod):
    del B_x
    return _impl(A_x, A_mem0, A_Wq, A_Wk, A_Wv, A_Wo, B_w1, B_b1, B_w2, B_b2, c, w_mod,
                 A_seg_len=int(A_seg_len))
```

```python
import functools

import jax
import jax.numpy as jnp
from jax import lax
import jax.experimental.pallas as pl
import jax.experimental.pallas.tpu as pltpu

F32 = jnp.float32
BF16 = jnp.bfloat16
U32 = jnp.uint32

_PROF = False


def _scope(name):
    import contextlib
    return jax.named_scope(name) if _PROF else contextlib.nullcontext()


_EPS = 1e-5
_NEG = -1e30


def _ln(x):
    m = jnp.mean(x, axis=-1, keepdims=True)
    xc = x - m
    v = jnp.mean(xc * xc, axis=-1, keepdims=True)
    return xc * lax.rsqrt(v + _EPS)


def _dot(a, b):
    return jnp.dot(a, b, preferred_element_type=F32)


def _dot_nt(a, b):
    return lax.dot_general(a, b, (((1,), (1,)), ((), ())), preferred_element_type=F32)


def _make_kernel(S, D, H, E, M, SEG, F):
    NSEG = S // SEG
    HE = H * E
    RIDE = 24
    XTRA = SEG - RIDE
    NX = NSEG * XTRA
    L = M + SEG
    LP = 48
    scale = float(E) ** -0.5
    NST = 4
    MODC = 2 * D

    def kernel(x_hbm, mem0_ref, wq_hbm, wk_hbm, wv_hbm, wo_hbm, w1_hbm, b1_ref,
               w2_hbm, b2_ref, c_ref, wmod_hbm, out_hbm,
               wq_s, wk_s, wv_s, wo_s, stage, w1_s, w2_s, wm_s, x_s, h_s, mod_s,
               qe_s, ke_s, ve_s, oe_s, ob_s, he_s, xe_s, sems, osems):
        def cp(src, dst, i):
            return pltpu.make_async_copy(src, dst, sems.at[i])

        NG = H // 8
        w3 = (wq_hbm, wk_hbm, wv_hbm)
        cp_w = [[cp(w3[m].at[:, pl.ds(g * 8, 8), :], stage.at[(m * NG + g) % NST], 20 + m * NG + g)
                 for g in range(NG)] for m in range(3)]
        cp_wm0 = cp(wmod_hbm.at[:, pl.ds(0, MODC)], wm_s, 0)
        cp_x = cp(x_hbm, x_s, 1)
        cp_xe = cp(x_hbm.at[:, pl.ds(RIDE, XTRA), :], xe_s, 2)
        cp_o = [cp(wo_hbm.at[:, pl.ds(j * 128, 128)], wo_s.at[j], 5 + j) for j in range(D // 128)]
        nd = 5 + D // 128
        cp_wm1 = cp(wmod_hbm.at[:, pl.ds(MODC, MODC)], wm_s, nd)
        cp_wm2 = cp(wmod_hbm.at[:, pl.ds(2 * MODC, MODC)], wm_s, nd + 1)
        cp_w1 = cp(w1_hbm, w1_s, nd + 2)
        cp_w2 = cp(w2_hbm, w2_s, nd + 3)

        cp_w[0][0].start()
        cp_wm0.start()
        cp_xe.start()

        c = c_ref[...].astype(F32).astype(BF16).astype(F32)
        sc = (c * jax.nn.sigmoid(c)).astype(BF16)
        sc = jnp.broadcast_to(sc, (8, D))

        def mod_chunk(j):
            r = _dot(sc, wm_s[...])
            mod_s[:, pl.ds(j * MODC, MODC)] = r.astype(BF16).astype(F32)

        def retile_chunk(slot, dst, g, t):
            src = stage.at[slot].bitcast(U32)
            blk = src.at[pl.ds(pl.multiple_of(t * 16, 16), 16)]
            r = pl.multiple_of(t * 8, 8)
            for hp in range(4):
                a = blk[pl.ds(0, 8, stride=2), hp, :]
                b = blk[pl.ds(1, 8, stride=2), hp, :]
                h = g * 8 + 2 * hp
                dst[h, pl.ds(r, 8), :] = (a & U32(0xFFFF)) | (b << 16)
                dst[h + 1, pl.ds(r, 8), :] = (a >> 16) | (b & U32(0xFFFF0000))

        def retile(slot, dst, g):
            def body(t, _):
                for u in range(4):
                    retile_chunk(slot, dst, g, t * 4 + u)
                return 0

            lax.fori_loop(0, D // 64, body, 0)

        def wtile(ref, h):
            return pltpu.bitcast(ref[h], BF16)

        HU = 4
        TU = (D // 16) // (8 // HU)

        def extra_proj(w_ref, dst, g, nxt):
            def body(i, _):
                for u in range(HU):
                    h = g * 8 + i * HU + u
                    dst[h] = _dot(he_s[...], wtile(w_ref, h)).astype(BF16)
                if nxt is not None:
                    for u in range(TU):
                        retile_chunk(nxt[0], nxt[1], nxt[2], i * TU + u)
                return 0

            lax.fori_loop(0, 8 // HU, body, 0)

        w_dst = (wq_s, wk_s, wv_s)
        e_dst = (qe_s, ke_s, ve_s)
        NU = 3 * NG
        unit = lambda u: (u // NG, u % NG)
        with _scope("wait_q"):
            cp_w[0][0].wait()
        for u in range(1, NST):
            cp_w[unit(u)[0]][unit(u)[1]].start()
        with _scope("retile_q"):
            retile(0, wq_s, 0)
        with _scope("wait_wm0"):
            cp_wm0.wait()
        mod_chunk(0)
        cp_x.start()
        sa = mod_s[0:1, 0:D]
        ca = mod_s[0:1, D:2 * D]

        def ln1(xv):
            return _ln(xv.astype(F32)) * (1.0 + ca) + sa

        cp_xe.wait()
        for blk in range(NX // 128):
            xv = xe_s[pl.ds(blk * 16, 16)].reshape(128, D)
            he_s[pl.ds(blk * 128, 128), :] = ln1(xv).astype(BF16)
        other = [cp_wm1] + cp_o + [cp_w1, cp_w2]
        with _scope("extra"):
            for u in range(NU):
                m, g = unit(u)
                nxt = None
                if u + 1 < NU:
                    m1, g1 = unit(u + 1)
                    cp_w[m1][g1].wait()
                    nxt = ((u + 1) % NST, w_dst[m1], g1)
                extra_proj(w_dst[m], e_dst[m], g, nxt)
                if u + NST < NU:
                    m2, g2 = unit(u + NST)
                    cp_w[m2][g2].start()
                elif other:
                    for d in other[:3]:
                        d.start()
                    other = other[3:]
        for d in other:
            d.start()
        for d in cp_o:
            d.wait()
        cp_wm1.wait()
        mod_chunk(1)
        cp_wm2.start()

        ga = mod_s[0:1, 2 * D:3 * D]
        cp_x.wait()
        h_s[pl.ds(0, RIDE), :] = ln1(x_s[0, pl.ds(0, RIDE), :])

        row = lax.broadcasted_iota(jnp.int32, (L, LP), 0)
        col = lax.broadcasted_iota(jnp.int32, (L, LP), 1)
        mask = (col < L) & ((row < M) | (col <= row))
        zpad = jnp.zeros((LP - L, E), F32)

        def softmax(s):
            s = jnp.where(mask, s * scale, _NEG)
            mx = jnp.max(s, axis=-1, keepdims=True)
            p = jnp.exp(s - mx)
            return (p / jnp.sum(p, axis=-1, keepdims=True)).astype(BF16)

        def step(s, mem):
            r0 = pl.multiple_of(s * SEG, SEG)
            lhs = jnp.concatenate([mem, h_s[pl.ds(r0, RIDE), :]], axis=0).astype(BF16)
            e0 = pl.multiple_of(s * XTRA, XTRA)
            s1 = jnp.minimum(s + 1, NSEG - 1)
            r1 = pl.multiple_of((s + 1) * SEG, SEG)
            h_s[pl.ds(r1, RIDE), :] = ln1(x_s[s1, pl.ds(0, RIDE), :])
            qa, ka, va, pa, oa = {}, {}, {}, {}, {}
            acc = [None]

            def do_qkv(h):
                q = _dot(lhs, wtile(wq_s, h))
                k = _dot(lhs, wtile(wk_s, h))
                v = _dot(lhs, wtile(wv_s, h))
                ke = ke_s[h, pl.ds(e0, XTRA), :].astype(F32)
                ve = ve_s[h, pl.ds(e0, XTRA), :].astype(F32)
                qe = qe_s[h, pl.ds(e0, XTRA), :].astype(F32)
                ka[h] = jnp.concatenate([k, ke, zpad], axis=0).astype(BF16)
                va[h] = jnp.concatenate([v, ve, zpad], axis=0).astype(BF16)
                qa[h] = jnp.concatenate([q, qe], axis=0).astype(BF16)

            def do_qk(h):
                pa[h] = softmax(_dot_nt(qa.pop(h), ka.pop(h)))

            def do_pv(h):
                o = _dot(pa.pop(h), va.pop(h))
                oe_s[pl.ds(e0, XTRA), h * E:(h + 1) * E] = o[M + RIDE:].astype(BF16)
                oa[h] = o[:M + RIDE].astype(BF16)

            def do_wo(h):
                o = oa.pop(h)
                r = jnp.concatenate(
                    [_dot(o, wo_s[j, h * E:(h + 1) * E, :]) for j in range(D // 128)], axis=1)
                acc[0] = r if acc[0] is None else acc[0] + r

            D1, D2 = 1, 3
            for t in range(2 * H):
                if t < H:
                    do_qkv(t)
                if 0 <= t - D1 < H:
                    do_qk(t - D1)
                if 0 <= t - D2 < H:
                    do_pv(t - D2)
                if t >= H:
                    do_wo(t - H)
            out = acc[0]
            h_s[pl.ds(r0, RIDE), :] = x_s[s, pl.ds(0, RIDE), :].astype(F32) + ga * out[M:]
            return out[0:M].astype(BF16).astype(F32)

        with _scope("loop"):
            lax.fori_loop(0, NSEG, step, mem0_ref[...].astype(F32))

        cp_w1.wait()
        cp_w2.wait()
        cp_wm2.wait()
        mod_chunk(2)

        for blk in range(NX // 128):
          with _scope("wo_extra"):
            segs = 128 // XTRA
            oe = oe_s[pl.ds(blk * 128, 128), :]
            out = jnp.concatenate([_dot(oe, wo_s[j]) for j in range(D // 128)], axis=1)
            for s in range(segs):
                r = (blk * segs + s) * SEG + RIDE
                h_s[pl.ds(r, XTRA), :] = (x_s[blk * segs + s, pl.ds(RIDE, XTRA), :].astype(F32)
                                          + ga * out[s * XTRA:(s + 1) * XTRA])

        sb = mod_s[0:1, 3 * D:4 * D]
        cb = mod_s[0:1, 4 * D:5 * D]
        gb = mod_s[0:1, 5 * D:6 * D]
        b2 = b2_ref[...].astype(F32)
        BM = 256
        FC = 512
        NB = S // BM

        def out_copy(i, slot):
            return pltpu.make_async_copy(
                ob_s.at[slot], out_hbm.at[pl.ds(pl.multiple_of(i * BM, BM), BM), :], osems.at[slot])

        def ffn_body(i, _):
            slot = i % 2
            r = pl.multiple_of(i * BM, BM)
            x1 = h_s[pl.ds(r, BM), :]
            hb = (_ln(x1) * (1.0 + cb) + sb).astype(BF16)
            acc = jnp.zeros((BM, D), F32)
            for f in range(F // FC):
                h1 = _dot(hb, w1_s[:, f * FC:(f + 1) * FC]) + b1_ref[:, f * FC:(f + 1) * FC].astype(F32)
                g = jax.nn.gelu(h1, approximate=True).astype(BF16)
                acc = acc + _dot(g, w2_s[f * FC:(f + 1) * FC, :])
            res = x1 + gb * (acc + b2)

            @pl.when(i >= 2)
            def _():
                out_copy(i - 2, slot).wait()

            ob_s[slot] = res.astype(BF16)
            out_copy(i, slot).start()
            return 0

        with _scope("ffn"):
            lax.fori_loop(0, NB, ffn_body, 0)
        out_copy(NB - 2, (NB - 2) % 2).wait()
        out_copy(NB - 1, (NB - 1) % 2).wait()

    return kernel


@functools.partial(jax.jit, static_argnames=("A_seg_len",))
def _impl(A_x, A_mem0, A_Wq, A_Wk, A_Wv, A_Wo, B_w1, B_b1, B_w2, B_b2, c, w_mod, A_seg_len):
    B, S, D = A_x.shape
    H, E = A_Wq.shape[1], A_Wq.shape[2]
    M = A_mem0.shape[1]
    F = B_w1.shape[1]
    SEG = A_seg_len
    assert B == 1 and E == 128 and M == 8 and SEG == 32
    NX = (S // SEG) * 8
    kernel = _make_kernel(S, D, H, E, M, SEG, F)
    any_spec = pl.BlockSpec(memory_space=pl.ANY)
    vmem_spec = pl.BlockSpec(memory_space=pltpu.VMEM)
    out = pl.pallas_call(
        kernel,
        out_shape=jax.ShapeDtypeStruct((S, D), A_x.dtype),
        in_specs=[any_spec, vmem_spec, any_spec, any_spec, any_spec, any_spec, any_spec,
                  vmem_spec, any_spec, vmem_spec, vmem_spec, any_spec],
        out_specs=any_spec,
        scratch_shapes=[
            pltpu.VMEM((H, D // 2, E), U32),
            pltpu.VMEM((H, D // 2, E), U32),
            pltpu.VMEM((H, D // 2, E), U32),
            pltpu.VMEM((D // 128, H * E, 128), BF16),
            pltpu.VMEM((4, D, 8, E), BF16),
            pltpu.VMEM((D, F), BF16),
            pltpu.VMEM((F, D), BF16),
            pltpu.VMEM((D, 2 * D), BF16),
            pltpu.VMEM((S // SEG, SEG, D), BF16),
            pltpu.VMEM((S + SEG, D), F32),
            pltpu.VMEM((8, 6 * D), F32),
            pltpu.VMEM((H, NX, E), BF16),
            pltpu.VMEM((H, NX, E), BF16),
            pltpu.VMEM((H, NX, E), BF16),
            pltpu.VMEM((NX, H * E), BF16),
            pltpu.VMEM((2, 256, D), BF16),
            pltpu.VMEM((NX, D), BF16),
            pltpu.VMEM((S // SEG, 8, D), BF16),
            pltpu.SemaphoreType.DMA((32,)),
            pltpu.SemaphoreType.DMA((2,)),
        ],
        compiler_params=pltpu.CompilerParams(vmem_limit_bytes=120 * 1024 * 1024),
    )(A_x.reshape(S // SEG, SEG, D), A_mem0.reshape(M, D),
      A_Wq, A_Wk, A_Wv,
      A_Wo.reshape(H * E, D), B_w1, B_b1.reshape(1, F), B_w2, B_b2.reshape(1, D), c, w_mod)
    return out.reshape(B, S, D)


def pallas_adaLN_cond__memory_aug_recurrent_mem_tr__dense_activation_gelu__prompt_kernel(
        A_x, A_mem0, A_Wq, A_Wk, A_Wv, A_Wo, A_seg_len, B_x, B_w1, B_b1, B_w2, B_b2, c, w_mod):
    del B_x
    return _impl(A_x, A_mem0, A_Wq, A_Wk, A_Wv, A_Wo, B_w1, B_b1, B_w2, B_b2, c, w_mod,
                 A_seg_len=int(A_seg_len))
```
